```python
import os as _os
_os.environ.setdefault("JAX_PLATFORMS", "cpu")
import jax
import jax.numpy as jnp

def _softmax(x, axis=-1):
    return jax.nn.softmax(x, axis=axis)
def _gelu(x):
    return jax.nn.gelu(x, approximate=True)
def _silu(x):
    return jax.nn.silu(x)
def _sigmoid(x):
    return jax.nn.sigmoid(x)
def _layernorm(x, axis=-1, eps=1e-5):
    m = jnp.mean(x, axis=axis, keepdims=True)
    v = jnp.var(x, axis=axis, keepdims=True)
    return (x - m) / jnp.sqrt(v + eps)
def _scatter_add(tgt, idx, src, axis=0):
    return tgt.at[idx].add(src)
def _segment_sum(src, seg, n):
    return jax.ops.segment_sum(src, seg, n)
class _Rng:
    def __init__(self, key):
        self._k = key
    def _next(self):
        self._k, sub = jax.random.split(self._k)
        return sub
    def normal(self, shape):
        return jax.random.normal(self._next(), shape, dtype=jnp.bfloat16)
    def randint(self, lo, hi, shape):
        return jax.random.randint(self._next(), shape, lo, hi, dtype=jnp.int32)
    def uniform(self, shape, lo=0.0, hi=1.0):
        return jax.random.uniform(self._next(), shape, jnp.bfloat16, lo, hi)
    def permutation(self, n):
        return jax.random.permutation(self._next(), n)


kernel_name = 'standalone__channel_attn_cbam__vision'

def setup_inputs():
    _rng = _Rng(jax.random.key(int.from_bytes(__import__("os").urandom(4), "little")))
    _w = (lambda a: (lambda t: t.astype(jnp.bfloat16) if jnp.issubdtype(t.dtype, jnp.floating) else t)(jnp.asarray(a)))
    H = W = 224
    C = 192
    r = max(C // 4, 1)
    return {
        "x": _w((lambda *s: _rng.normal(s) * 0.2)(1, H, W, C) + (lambda *s: _rng.normal(s) * 0.2)(1, 1, 1, C) * 2.0),
        "w1": _w((lambda *s: _rng.normal(s) * 0.2)(C, r)),
        "w2": _w((lambda *s: _rng.normal(s) * 0.2)(r, C)),
    }

def reference(x, w1, w2):
    B, H, W, C = x.shape
    xf = x.reshape(B, H * W, C)
    gap = jnp.mean(xf, 1)
    gmp = jnp.amax(xf, 1)
    h_a = gap @ w1
    h_a = h_a * (lambda x, dt: x.astype(dt))(h_a > 0, h_a.dtype)
    h_m = gmp @ w1
    h_m = h_m * (lambda x, dt: x.astype(dt))(h_m > 0, h_m.dtype)
    scale = _sigmoid(h_a @ w2 + h_m @ w2)
    return x * scale[:, None, None, :]
```

```python
import jax
import jax.numpy as jnp
from jax import lax
import jax.experimental.pallas as pl
import jax.experimental.pallas.tpu as pltpu

F32, BF16 = jnp.float32, jnp.bfloat16

H, W, C, HID = 224, 224, 192, 48
G = 16
T = C // G
A, HS = 7, 32
TQ = 3
LANES = 128
HALF = LANES // 2

BULK = (96, 64, 32)
REST = (20, 8, 4)
LAST = (26, 4, 2)
N_PRE = 1


def _reads():
    out, h0 = [], 0
    for n in BULK:
        out.append((h0, n, 0, T))
        h0 += n
    for sizes, t0, nt in ((REST, 1, T - 1), (LAST, 0, 1)):
        h0 = sum(BULK)
        for n in sizes:
            out.append((h0, n, t0, nt))
            h0 += n
        assert h0 == H
    return out


READS = _reads()
I_REST_END = len(BULK) + len(REST) - 1


def _rb(v):
    return v.astype(BF16).astype(F32)


def _kernel(x_hbm, w1t_hbm, w2_hbm, o_hbm,
            xbuf, obuf, w1t_v, w2_v, w1d_v, w2d_v, acc_s, acc_m, p_v, h_v, scale_v,
            sem_wr):

    def layer1_partial(s, m, t0, nt):
        lane = lax.broadcasted_iota(jnp.int32, (nt, G, LANES), 2)
        gap = _rb(jnp.sum(s, axis=2, keepdims=True) * (1.0 / (H * W)))
        gmp = jnp.max(m, axis=2, keepdims=True)
        g = jnp.where(lane < HALF,
                      jnp.broadcast_to(gap, (nt, G, LANES)),
                      jnp.broadcast_to(gmp, (nt, G, LANES)))
        return jnp.sum((g * w1d_v[pl.ds(t0, nt)]).reshape(nt * 2, 8, LANES), axis=0)

    def accumulate(h0, n, t0, nt, init):
        ts = pl.ds(t0, nt)
        if init is None:
            v = xbuf[h0, ts].astype(F32)
            init, lo = (v, v), 1
        else:
            lo = 0

        def body(k, carry):
            s, m = carry
            v = xbuf[h0 + k, ts].astype(F32)
            return s + v, jnp.maximum(m, v)

        if n - lo <= 4:
            for k in range(lo, n):
                init = body(k, init)
            return init
        return lax.fori_loop(lo, n, body, init, unroll=2)

    def scale_for(t0, nt, h_a, h_m):
        w = w2d_v[pl.ds(t0, nt)].reshape(nt * 2, 8, LANES)
        za = _rb(jnp.sum(w * h_a[None], axis=2, keepdims=True))
        zm = _rb(jnp.sum(w * h_m[None], axis=2, keepdims=True))
        z = jnp.broadcast_to(_rb(za + zm), (nt * 2, 8, LANES))
        sc = _rb(1.0 / _rb(1.0 + _rb(jnp.exp(-z))))
        return sc.reshape(nt, G, LANES)

    def widen(sc):
        return jnp.concatenate([sc, sc[:, :, :W - LANES]], axis=2)

    def emit(hs, t0, nt, scw):
        ts = pl.ds(t0, nt)
        for a in range(A):
            obuf[a, hs, ts] = (xbuf[a * HS + hs, ts].astype(F32) * scw).astype(BF16)
        pltpu.make_async_copy(obuf.at[:, hs, ts], o_hbm.at[:, hs, ts], sem_wr).start()

    def main(sem_rd):
        def rd_copy(i):
            h0, n, t0, nt = READS[i]
            return pltpu.make_async_copy(
                x_hbm.at[pl.ds(h0, n), pl.ds(t0, nt)],
                xbuf.at[pl.ds(h0, n), pl.ds(t0, nt)],
                sem_rd.at[i])

        cw1 = pltpu.make_async_copy(w1t_hbm, w1t_v, sem_wr)
        cw2 = pltpu.make_async_copy(w2_hbm, w2_v, sem_wr)
        cw1.start()
        cw2.start()
        rd_copy(0).start()

        def zero_body(k, carry):
            h_v[k] = jnp.zeros((8, LANES), F32)
            return carry
        lax.fori_loop(0, 2, zero_body, 0)

        for i in range(1, len(READS)):
            rd_copy(i).start()

        carry, p = None, None
        for i, (h0, n, t0, nt) in enumerate(READS):
            rd_copy(i).wait()
            for b0 in range(t0, t0 + nt, TQ):
                nb = min(TQ, t0 + nt - b0)
                if i == 0:
                    init = None
                elif carry is not None:
                    init = carry
                else:
                    init = (acc_s[pl.ds(b0, nb)], acc_m[pl.ds(b0, nb)])
                s, m = accumulate(h0, n, b0, nb, init)
                if i == I_REST_END:
                    pp = layer1_partial(s, m, b0, nb)
                    p = pp if p is None else p + pp
                elif i > I_REST_END:
                    carry = (s, m)
                else:
                    acc_s[pl.ds(b0, nb)] = s
                    acc_m[pl.ds(b0, nb)] = m
            if i == 0:
                cw1.wait()
                cw2.wait()
                pad = jnp.zeros((HALF - HID, C), F32)
                w1f = w1t_v[...].astype(F32)
                w2f = w2_v[...].astype(F32)
                w1d_v[...] = jnp.concatenate([w1f, pad, w1f, pad], axis=0).T.reshape(T, G, LANES)
                w2d_v[...] = jnp.concatenate([w2f, pad, w2f, pad], axis=0).T.reshape(T, G, LANES)
            if i == I_REST_END:
                p_v[...] = p

        p = p_v[...] + layer1_partial(carry[0], carry[1], 0, 1)
        hp = jnp.broadcast_to(_rb(jnp.sum(p, axis=0, keepdims=True)), (8, LANES))
        hr = jnp.where(hp > 0, hp, hp * 0.0)
        lane = lax.broadcasted_iota(jnp.int32, (8, LANES), 1)
        h_a = jnp.where(lane < HID, hr, 0.0)
        h_m = jnp.where((lane >= HALF) & (lane < HALF + HID), hr, 0.0)
        h_v[0] = h_a
        h_v[1] = h_m

        sc0 = scale_for(0, 1, h_a, h_m)
        scale_v[pl.ds(0, 1)] = sc0
        scw0 = widen(sc0)
        emit(0, 0, 1, scw0)

        def pre_body(hs, carry):
            emit(hs, 0, 1, scw0)
            return carry
        lax.fori_loop(1, 1 + N_PRE, pre_body, 0)

        scale_v[pl.ds(1, T - 1)] = scale_for(1, T - 1, h_v[0], h_v[1])

        def head_body(hs, carry):
            emit(hs, 1, TQ - 1, widen(scale_v[pl.ds(1, TQ - 1)]))
            for t0 in range(TQ, T, TQ):
                emit(hs, t0, TQ, widen(scale_v[pl.ds(t0, TQ)]))
            return carry
        lax.fori_loop(0, 1 + N_PRE, head_body, 0)

        def main_body(hs, carry):
            for t0 in range(0, T, TQ):
                emit(hs, t0, TQ, widen(scale_v[pl.ds(t0, TQ)]))
            return carry
        lax.fori_loop(1 + N_PRE, HS, main_body, 0)

    pl.run_scoped(main, pltpu.SemaphoreType.DMA((len(READS),)))
    pltpu.make_async_copy(obuf, o_hbm, sem_wr).wait()


@jax.jit
def pallas_standalone__channel_attn_cbam__vision_kernel(
    x: jax.Array,
    w1: jax.Array,
    w2: jax.Array,
):
    assert x.shape == (1, H, W, C) and w1.shape == (C, HID) and w2.shape == (HID, C)
    xt = jnp.transpose(x, (0, 1, 3, 2)).reshape(H, T, G, W)
    out = pl.pallas_call(
        _kernel,
        out_shape=jax.ShapeDtypeStruct((A, HS, T, G, W), x.dtype),
        in_specs=[pl.BlockSpec(memory_space=pl.ANY)] * 3,
        out_specs=pl.BlockSpec(memory_space=pl.ANY),
        scratch_shapes=[
            pltpu.VMEM((H, T, G, W), BF16),
            pltpu.VMEM((A, HS, T, G, W), BF16),
            pltpu.VMEM((HID, C), BF16),
            pltpu.VMEM((HID, C), BF16),
            pltpu.VMEM((T, G, LANES), F32),
            pltpu.VMEM((T, G, LANES), F32),
            pltpu.VMEM((T, G, W), F32),
            pltpu.VMEM((T, G, W), F32),
            pltpu.VMEM((8, LANES), F32),
            pltpu.VMEM((2, 8, LANES), F32),
            pltpu.VMEM((T, G, LANES), F32),
            pltpu.SemaphoreType.DMA(()),
        ],
        compiler_params=pltpu.CompilerParams(vmem_limit_bytes=100 * 1024 * 1024),
    )(xt, w1.T, w2)
    return jnp.transpose(out.reshape(1, H, C, W), (0, 1, 3, 2))
```

```python
import jax
import jax.numpy as jnp
from jax import lax
import jax.experimental.pallas as pl
import jax.experimental.pallas.tpu as pltpu

F32, BF16 = jnp.float32, jnp.bfloat16

H, W, C, HID = 224, 224, 192, 48
G = 16
T = C // G
TQ = 3
A, HS = 7, 32
LANES = 128
HALF = LANES // 2

READS = (
    (192, 32, 1, T - 1),
    (0, 96, 0, T), (96, 56, 0, T), (152, 24, 0, T), (176, 10, 0, T), (186, 4, 0, T), (190, 2, 0, T),
    (192, 20, 0, 1), (212, 8, 0, 1), (220, 4, 0, 1),
)
W_AFTER = 2
N_PRE = 2


def _plan():
    rows, plan = [0] * T, []
    for _, n, t0, nt in READS:
        state = {t: (rows[t] == 0, rows[t] + n == H) for t in range(t0, t0 + nt)}
        blocks, t = [], t0
        while t < t0 + nt:
            nb = 1
            while nb < TQ and t + nb < t0 + nt and state[t + nb] == state[t]:
                nb += 1
            blocks.append((t, nb) + state[t])
            t += nb
        for t in state:
            rows[t] += n
        plan.append(blocks)
    assert rows == [H] * T
    return plan


PLAN = _plan()


def _rb(v):
    return v.astype(BF16).astype(F32)


def _body(x_hbm, w1t_hbm, w2_hbm, o_hbm,
          xbuf, obuf, w1t_v, w2_v, w1d_v, w2d_v, acc_s, acc_m, p0_v, scale_v,
          sem_rd, sem_wr):

    def accumulate(h0, n, t0, nt, init):
        ts = pl.ds(t0, nt)
        lo = 0
        if init is None:
            v = xbuf[h0, ts].astype(F32)
            init, lo = (v, v), 1

        def step(k, carry):
            s, m = carry
            v = xbuf[h0 + k, ts].astype(F32)
            return s + v, jnp.maximum(m, v)

        if n - lo > 8:
            return lax.fori_loop(lo, n, step, init, unroll=4)
        for k in range(lo, n):
            init = step(k, init)
        return init

    def layer1_partial(s, m, t0, nt):
        lane = lax.broadcasted_iota(jnp.int32, (nt, G, LANES), 2)
        gap = _rb(jnp.sum(s, axis=2, keepdims=True) * (1.0 / (H * W)))
        gmp = jnp.max(m, axis=2, keepdims=True)
        g = jnp.where(lane < HALF,
                      jnp.broadcast_to(gap, (nt, G, LANES)),
                      jnp.broadcast_to(gmp, (nt, G, LANES)))
        return jnp.sum((g * w1d_v[pl.ds(t0, nt)]).reshape(nt * 2, 8, LANES), axis=0)

    def scale_for(t0, nt, h_a, h_m):
        w = w2d_v[pl.ds(t0, nt)].reshape(nt * 2, 8, LANES)
        za = _rb(jnp.sum(w * h_a[None], axis=2, keepdims=True))
        zm = _rb(jnp.sum(w * h_m[None], axis=2, keepdims=True))
        z = jnp.broadcast_to(_rb(za + zm), (nt * 2, 8, LANES))
        sc = _rb(1.0 / _rb(1.0 + _rb(jnp.exp(-z))))
        return sc.reshape(nt, G, LANES)

    def emit(hs, t0, nt, sc):
        ts = pl.ds(t0, nt)
        scw = jnp.concatenate([sc, sc[:, :, :W - LANES]], axis=2)
        for a in range(A):
            obuf[a, hs, ts] = (xbuf[a * HS + hs, ts].astype(F32) * scw).astype(BF16)
        pltpu.make_async_copy(obuf.at[:, hs, ts], o_hbm.at[:, hs, ts], sem_wr).start()

    def rd_copy(i):
        h0, n, t0, nt = READS[i]
        return pltpu.make_async_copy(
            x_hbm.at[pl.ds(h0, n), pl.ds(t0, nt)],
            xbuf.at[pl.ds(h0, n), pl.ds(t0, nt)],
            sem_rd.at[i])

    cw1 = pltpu.make_async_copy(w1t_hbm, w1t_v, sem_wr)
    cw2 = pltpu.make_async_copy(w2_hbm, w2_v, sem_wr)
    cw1.start()
    cw2.start()
    rd_copy(0).start()

    def zero_step(k, carry):
        p0_v[k] = jnp.zeros((8, LANES), F32)
        return carry
    lax.fori_loop(0, 2, zero_step, 0)

    for i in range(1, len(READS)):
        rd_copy(i).start()

    p = None
    held = None
    for i, (h0, n, _, _) in enumerate(READS):
        rd_copy(i).wait()
        for b0, nb, first, done in PLAN[i]:
            if first:
                init = None
            elif held is not None and held[0] == (b0, nb):
                init, held = held[1], None
            else:
                init = (acc_s[pl.ds(b0, nb)], acc_m[pl.ds(b0, nb)])
            s, m = accumulate(h0, n, b0, nb, init)
            if done:
                p = (p0_v[0] + p0_v[1] if p is None else p) + layer1_partial(s, m, b0, nb)
            elif len(PLAN[i]) == 1 and [b[:2] for b in PLAN[i + 1]] == [(b0, nb)]:
                held = ((b0, nb), (s, m))
            else:
                acc_s[pl.ds(b0, nb)] = s
                acc_m[pl.ds(b0, nb)] = m
        if i == W_AFTER:
            cw1.wait()
            cw2.wait()
            pad = jnp.zeros((HALF - HID, C), F32)
            w1f = w1t_v[...].astype(F32)
            w2f = w2_v[...].astype(F32)
            w1d_v[...] = jnp.concatenate([w1f, pad, w1f, pad], axis=0).T.reshape(T, G, LANES)
            w2d_v[...] = jnp.concatenate([w2f, pad, w2f, pad], axis=0).T.reshape(T, G, LANES)

    hp = jnp.broadcast_to(_rb(jnp.sum(p, axis=0, keepdims=True)), (8, LANES))
    hr = jnp.where(hp > 0, hp, hp * 0.0)
    lane = lax.broadcasted_iota(jnp.int32, (8, LANES), 1)
    h_a = jnp.where(lane < HID, hr, 0.0)
    h_m = jnp.where((lane >= HALF) & (lane < HALF + HID), hr, 0.0)

    sc0 = scale_for(0, 1, h_a, h_m)
    scale_v[pl.ds(0, 1)] = sc0
    for hs in range(N_PRE):
        emit(hs, 0, 1, sc0)
    scale_v[pl.ds(1, T - 1)] = scale_for(1, T - 1, h_a, h_m)

    def head_step(hs, carry):
        emit(hs, 1, TQ - 1, scale_v[pl.ds(1, TQ - 1)])
        for t0 in range(TQ, T, TQ):
            emit(hs, t0, TQ, scale_v[pl.ds(t0, TQ)])
        return carry
    lax.fori_loop(0, N_PRE, head_step, 0)

    def main_step(hs, carry):
        for t0 in range(0, T, TQ):
            emit(hs, t0, TQ, scale_v[pl.ds(t0, TQ)])
        return carry
    lax.fori_loop(N_PRE, HS, main_step, 0)

    pltpu.make_async_copy(obuf, o_hbm, sem_wr).wait()


def _kernel(*refs):
    pl.run_scoped(
        lambda sem_rd, sem_wr: _body(*refs, sem_rd, sem_wr),
        pltpu.SemaphoreType.DMA((len(READS),)),
        pltpu.SemaphoreType.DMA(()),
    )


@jax.jit
def pallas_standalone__channel_attn_cbam__vision_kernel(
    x: jax.Array,
    w1: jax.Array,
    w2: jax.Array,
):
    assert x.shape == (1, H, W, C) and w1.shape == (C, HID) and w2.shape == (HID, C)
    xt = jnp.transpose(x, (0, 1, 3, 2)).reshape(H, T, G, W)
    out = pl.pallas_call(
        _kernel,
        out_shape=jax.ShapeDtypeStruct((A, HS, T, G, W), BF16),
        in_specs=[pl.BlockSpec(memory_space=pl.ANY)] * 3,
        out_specs=pl.BlockSpec(memory_space=pl.ANY),
        scratch_shapes=[
            pltpu.VMEM((H, T, G, W), BF16),
            pltpu.VMEM((A, HS, T, G, W), BF16),
            pltpu.VMEM((HID, C), BF16),
            pltpu.VMEM((HID, C), BF16),
            pltpu.VMEM((T, G, LANES), F32),
            pltpu.VMEM((T, G, LANES), F32),
            pltpu.VMEM((T, G, W), F32),
            pltpu.VMEM((T, G, W), F32),
            pltpu.VMEM((2, 8, LANES), F32),
            pltpu.VMEM((T, G, LANES), F32),
        ],
        compiler_params=pltpu.CompilerParams(vmem_limit_bytes=64 * 1024 * 1024),
    )(xt, w1.T, w2)
    return jnp.transpose(out.reshape(1, H, C, W), (0, 1, 3, 2))
```

```python
import jax
import jax.numpy as jnp
from jax import lax
import jax.experimental.pallas as pl
import jax.experimental.pallas.tpu as pltpu

F32, BF16 = jnp.float32, jnp.bfloat16

H, W, C, HID = 224, 224, 192, 48
G = 16
T = C // G
TQ = 3
A, HS = 7, 32
LANES = 128
HALF = LANES // 2

READS = (
    (208, 16, 2, T - 2),
    (0, 104, 0, T), (104, 60, 0, T), (164, 28, 0, T), (192, 10, 0, T), (202, 4, 0, T), (206, 2, 0, T),
    (208, 11, 0, 2), (219, 4, 0, 2), (223, 1, 0, 2),
)
W_AFTER = 2
N_PRE = 2


def _plan():
    rows, plan = [0] * T, []
    for _, n, t0, nt in READS:
        state = {t: (rows[t] == 0, rows[t] + n == H) for t in range(t0, t0 + nt)}
        blocks, t = [], t0
        while t < t0 + nt:
            nb = 1
            while nb < TQ and t + nb < t0 + nt and state[t + nb] == state[t]:
                nb += 1
            blocks.append((t, nb) + state[t])
            t += nb
        for t in state:
            rows[t] += n
        plan.append(blocks)
    assert rows == [H] * T
    return plan


PLAN = _plan()


def _rb(v):
    return v.astype(BF16).astype(F32)


def _body(x_hbm, w1t_hbm, w2_hbm, o_hbm,
          xbuf, obuf, w1t_v, w2_v, w1d_v, w2d_v, acc_s, acc_m, p0_v, scale_v,
          sem_rd, sem_wr):

    def accumulate(h0, n, t0, nt, init):
        ts = pl.ds(t0, nt)
        lo = 0
        if init is None:
            v = xbuf[h0, ts].astype(F32)
            init, lo = (v, v), 1

        def step(k, carry):
            s, m = carry
            v = xbuf[h0 + k, ts].astype(F32)
            return s + v, jnp.maximum(m, v)

        if n - lo > 8:
            return lax.fori_loop(lo, n, step, init, unroll=4)
        for k in range(lo, n):
            init = step(k, init)
        return init

    def layer1_partial(s, m, t0, nt):
        lane = lax.broadcasted_iota(jnp.int32, (nt, G, LANES), 2)
        gap = _rb(jnp.sum(s, axis=2, keepdims=True) * (1.0 / (H * W)))
        gmp = jnp.max(m, axis=2, keepdims=True)
        g = jnp.where(lane < HALF,
                      jnp.broadcast_to(gap, (nt, G, LANES)),
                      jnp.broadcast_to(gmp, (nt, G, LANES)))
        return jnp.sum((g * w1d_v[pl.ds(t0, nt)]).reshape(nt * 2, 8, LANES), axis=0)

    def scale_for(t0, nt, hid):
        shape = (nt * 2, 8, LANES)
        lane = lax.broadcasted_iota(jnp.int32, shape, 2)
        q = w2d_v[pl.ds(t0, nt)].reshape(shape) * hid[None]
        qa = jnp.where(lane < HID, q, 0.0)
        qm = jnp.where((lane >= HALF) & (lane < HALF + HID), q, 0.0)
        za = _rb(jnp.sum(qa, axis=2, keepdims=True))
        zm = _rb(jnp.sum(qm, axis=2, keepdims=True))
        z = jnp.broadcast_to(_rb(za + zm), shape)
        sc = _rb(1.0 / _rb(1.0 + _rb(jnp.exp(-z))))
        return sc.reshape(nt, G, LANES)

    def emit(hs, t0, nt, sc):
        ts = pl.ds(t0, nt)
        scw = jnp.concatenate([sc, sc[:, :, :W - LANES]], axis=2)
        for a in range(A):
            obuf[a, hs, ts] = (xbuf[a * HS + hs, ts].astype(F32) * scw).astype(BF16)
        pltpu.make_async_copy(obuf.at[:, hs, ts], o_hbm.at[:, hs, ts], sem_wr).start()

    def rd_copy(i):
        h0, n, t0, nt = READS[i]
        return pltpu.make_async_copy(
            x_hbm.at[pl.ds(h0, n), pl.ds(t0, nt)],
            xbuf.at[pl.ds(h0, n), pl.ds(t0, nt)],
            sem_rd.at[i])

    cw1 = pltpu.make_async_copy(w1t_hbm, w1t_v, sem_wr)
    cw2 = pltpu.make_async_copy(w2_hbm, w2_v, sem_wr)
    rd_copy(0).start()
    cw1.start()
    cw2.start()

    def zero_step(k, carry):
        p0_v[k] = jnp.zeros((8, LANES), F32)
        return carry
    lax.fori_loop(0, 2, zero_step, 0)

    for i in range(1, len(READS)):
        rd_copy(i).start()

    p = None
    held = None
    for i, (h0, n, _, _) in enumerate(READS):
        rd_copy(i).wait()
        for b0, nb, first, done in PLAN[i]:
            if first:
                init = None
            elif held is not None and held[0] == (b0, nb):
                init, held = held[1], None
            else:
                init = (acc_s[pl.ds(b0, nb)], acc_m[pl.ds(b0, nb)])
            s, m = accumulate(h0, n, b0, nb, init)
            if done:
                p = (p0_v[0] + p0_v[1] if p is None else p) + layer1_partial(s, m, b0, nb)
            elif len(PLAN[i]) == 1 and [b[:2] for b in PLAN[i + 1]] == [(b0, nb)]:
                held = ((b0, nb), (s, m))
            else:
                acc_s[pl.ds(b0, nb)] = s
                acc_m[pl.ds(b0, nb)] = m
        if i == W_AFTER:
            cw1.wait()
            cw2.wait()
            pad = jnp.zeros((HALF - HID, C), F32)
            w1f = w1t_v[...].astype(F32)
            w2f = w2_v[...].astype(F32)
            w1d_v[...] = jnp.concatenate([w1f, pad, w1f, pad], axis=0).T.reshape(T, G, LANES)
            w2d_v[...] = jnp.concatenate([w2f, pad, w2f, pad], axis=0).T.reshape(T, G, LANES)

    hp = jnp.broadcast_to(_rb(jnp.sum(p, axis=0, keepdims=True)), (8, LANES))
    hid = jnp.where(hp > 0, hp, hp * 0.0)

    sc0 = scale_for(0, 1, hid)
    scale_v[pl.ds(0, 1)] = sc0
    for hs in range(N_PRE):
        emit(hs, 0, 1, sc0)
    scale_v[pl.ds(1, T - 1)] = scale_for(1, T - 1, hid)

    def head_step(hs, carry):
        emit(hs, 1, TQ - 1, scale_v[pl.ds(1, TQ - 1)])
        for t0 in range(TQ, T, TQ):
            emit(hs, t0, TQ, scale_v[pl.ds(t0, TQ)])
        return carry
    lax.fori_loop(0, N_PRE, head_step, 0)

    def main_step(hs, carry):
        for t0 in range(0, T, TQ):
            emit(hs, t0, TQ, scale_v[pl.ds(t0, TQ)])
        return carry
    lax.fori_loop(N_PRE, HS, main_step, 0)

    pltpu.make_async_copy(obuf, o_hbm, sem_wr).wait()


def _kernel(*refs):
    pl.run_scoped(
        lambda sem_rd, sem_wr: _body(*refs, sem_rd, sem_wr),
        pltpu.SemaphoreType.DMA((len(READS),)),
        pltpu.SemaphoreType.DMA(()),
    )


@jax.jit
def pallas_standalone__channel_attn_cbam__vision_kernel(
    x: jax.Array,
    w1: jax.Array,
    w2: jax.Array,
):
    assert x.shape == (1, H, W, C) and w1.shape == (C, HID) and w2.shape == (HID, C)
    xt = jnp.transpose(x, (0, 1, 3, 2)).reshape(H, T, G, W)
    out = pl.pallas_call(
        _kernel,
        out_shape=jax.ShapeDtypeStruct((A, HS, T, G, W), BF16),
        in_specs=[pl.BlockSpec(memory_space=pl.ANY)] * 3,
        out_specs=pl.BlockSpec(memory_space=pl.ANY),
        scratch_shapes=[
            pltpu.VMEM((H, T, G, W), BF16),
            pltpu.VMEM((A, HS, T, G, W), BF16),
            pltpu.VMEM((HID, C), BF16),
            pltpu.VMEM((HID, C), BF16),
            pltpu.VMEM((T, G, LANES), F32),
            pltpu.VMEM((T, G, LANES), F32),
            pltpu.VMEM((T, G, W), F32),
            pltpu.VMEM((T, G, W), F32),
            pltpu.VMEM((2, 8, LANES), F32),
            pltpu.VMEM((T, G, LANES), F32),
        ],
        compiler_params=pltpu.CompilerParams(vmem_limit_bytes=64 * 1024 * 1024),
    )(xt, w1.T, w2)
    return jnp.transpose(out.reshape(1, H, C, W), (0, 1, 3, 2))
```
